```python
import os as _os
_os.environ.setdefault("JAX_PLATFORMS", "cpu")
import jax
import jax.numpy as jnp

def _softmax(x, axis=-1):
    return jax.nn.softmax(x, axis=axis)
def _gelu(x):
    return jax.nn.gelu(x, approximate=True)
def _silu(x):
    return jax.nn.silu(x)
def _sigmoid(x):
    return jax.nn.sigmoid(x)
def _layernorm(x, axis=-1, eps=1e-5):
    m = jnp.mean(x, axis=axis, keepdims=True)
    v = jnp.var(x, axis=axis, keepdims=True)
    return (x - m) / jnp.sqrt(v + eps)
def _scatter_add(tgt, idx, src, axis=0):
    return tgt.at[idx].add(src)
def _segment_sum(src, seg, n):
    return jax.ops.segment_sum(src, seg, n)
class _Rng:
    def __init__(self, key):
        self._k = key
    def _next(self):
        self._k, sub = jax.random.split(self._k)
        return sub
    def normal(self, shape):
        return jax.random.normal(self._next(), shape, dtype=jnp.bfloat16)
    def randint(self, lo, hi, shape):
        return jax.random.randint(self._next(), shape, lo, hi, dtype=jnp.int32)
    def uniform(self, shape, lo=0.0, hi=1.0):
        return jax.random.uniform(self._next(), shape, jnp.bfloat16, lo, hi)
    def permutation(self, n):
        return jax.random.permutation(self._next(), n)


kernel_name = 'sequential_preLN__softmax_full_mha__glu_gated_swiglu__prompt'

def setup_inputs():
    _rng = _Rng(jax.random.key(int.from_bytes(__import__("os").urandom(4), "little")))
    _w = (lambda a: (lambda t: t.astype(jnp.bfloat16) if jnp.issubdtype(t.dtype, jnp.floating) else t)(jnp.asarray(a)))
    def _A_setup():
        B, S, D = 1, 2048, 512
        return {
            "x": _w((lambda *s: _rng.normal(s) * 0.05)(B, S, D)),
            "wqkv": _w((lambda *s: _rng.normal(s) * 0.05)(D, 3 * D)),
            "wo": _w((lambda *s: _rng.normal(s) * 0.05)(D, D)),
        }
    _A_in = _A_setup()

    def _B_setup():
        B, S, D, F = 1, 2048, 512, 1376
        return {
            "x": _w((lambda *s: _rng.normal(s) * 0.05)(B, S, D)),
            "w1": _w((lambda *s: _rng.normal(s) * 0.05)(D, F) * (2.0 / D) ** 0.5),
            "w3": _w((lambda *s: _rng.normal(s) * 0.05)(D, F) * (2.0 / D) ** 0.5),
            "w2": _w((lambda *s: _rng.normal(s) * 0.05)(F, D) * (2.0 / F) ** 0.5),
        }
    _B_in = _B_setup()

    return {
        "A_x": _A_in["x"],
        "A_wqkv": _A_in["wqkv"],
        "A_wo": _A_in["wo"],
        "B_x": _B_in["x"],
        "B_w1": _B_in["w1"],
        "B_w3": _B_in["w3"],
        "B_w2": _B_in["w2"],
    }

def reference(A_x, A_wqkv, A_wo, B_x, B_w1, B_w3, B_w2):
    def _A_ref(x, wqkv, wo):
        B, S, D = x.shape
        H = 32; Dh = D // H
        qkv = (lambda x, *d: x.transpose(*d))((x @ wqkv).reshape(B, S, 3, H, Dh), 2, 0, 3, 1, 4)
        q, k, v = qkv[0], qkv[1], qkv[2]
        scale = Dh ** -0.5
        scores = jnp.einsum("bhqd,bhkd->bhqk", q, k) * scale
        p = _softmax(scores, axis=-1)
        o = jnp.einsum("bhqk,bhkd->bhqd", p, v)
        return (lambda x, *d: x.transpose(*d))(o, 0, 2, 1, 3).reshape(B, S, D) @ wo

    def _B_ref(x, w1, w3, w2):
        gate = jnp.einsum("bsd,df->bsf", x, w1)
        up = jnp.einsum("bsd,df->bsf", x, w3)
        h = _silu(gate) * up
        out = jnp.einsum("bsf,fd->bsd", h, w2)
        return out

    x = A_x
    h = x + _A_ref(_layernorm(x, axis=-1), A_wqkv, A_wo)
    h2 = h + _B_ref(_layernorm(h, axis=-1), B_w1, B_w3, B_w2)
    return h2
```

```python
import jax
import jax.numpy as jnp
from jax import lax
import jax.experimental.pallas as pl
import jax.experimental.pallas.tpu as pltpu

S = 2048
D = 512
H = 32
DH = D // H
F = 1376
EPS = 1e-5

TQ = 512
NQ = S // TQ
CK = 256
PK = 128
NC = S // CK
HB = 2
TF = 128

LOG2E = 1.4426950408889634
Q_SCALE = (DH ** -0.5) * LOG2E

QMAX = 3567.0
ROUND_MAGIC = 12582912.0
ROUND_BIAS = 0x4B400000 - 528
ACC_UNIT = 1024.0

LOGIT_LIMIT = 80.0
V_HI = 2.0 ** 20
V_LO = 2.0 ** -20

_NT = (((1,), (1,)), ((), ()))


def _layernorm_f32(x):
    mu = jnp.mean(x, axis=-1, keepdims=True)
    xc = x - mu
    var = jnp.mean(xc * xc, axis=-1, keepdims=True)
    return xc * lax.rsqrt(var + EPS)


def _fold_lanes(x, op):
    parts = [x[:, c:c + 128] for c in range(0, x.shape[1], 128)]
    while len(parts) > 1:
        parts = [op(parts[i], parts[i + 1]) for i in range(0, len(parts), 2)]
    return parts[0]


def _splat_max(a):
    t = _fold_lanes(jnp.maximum(a[0:8], a[8:16]), jnp.maximum)
    t = jnp.broadcast_to(jnp.max(t, axis=1, keepdims=True), (8, 128))
    return jnp.max(t, axis=0, keepdims=True)


def _recip(x):
    r = pl.reciprocal(x, approx=True)
    return r * (2.0 - x * r)


def _limbs(x):
    z = lax.bitcast_convert_type(x + ROUND_MAGIC, jnp.int32) - ROUND_BIAS
    t = z >> 5
    u1, u0 = t & 31, z & 31
    return t & -32, z >> 10, u1 - 16, u0 - 16, (u1 - 14) >> 2, (u0 - 12) >> 3


def _limb_words(x):
    z = lax.bitcast_convert_type(x + ROUND_MAGIC, jnp.int32) - (ROUND_BIAS - 3072)
    zb = [z[:, b * 128:(b + 1) * 128] for b in range(4)]

    def bytes_of(f):
        u0 = f & 0x001F001F
        u1 = (f >> 5) & 0x001F001F
        t2 = (f >> 10) & 0x00070007
        byte = 0x00FF00FF
        return (((t2 + 0x00050005) & 0x00070007) << 5,
                (t2 + 0x00FD00FD) & byte,
                (u1 + 0x00F000F0) & byte,
                (u0 + 0x00F000F0) & byte,
                ((((u1 + 0x00020002) >> 2) & 0x000F000F) + 0x00FC00FC) & byte,
                ((((u0 + 0x00040004) >> 3) & 0x00070007) + 0x00FE00FE) & byte)

    even = bytes_of(zb[0] | (zb[2] << 16))
    odd = bytes_of(zb[1] | (zb[3] << 16))
    return [e | (o << 8) for e, o in zip(even, odd)]


def _kernel(x_hbm, wqkv_hbm, wo_hbm, w1_hbm, w3_hbm, w2_hbm, out_hbm,
            x_v, wqkv_v, wo_v, w1_v, w3_v, w2_v, wt_scr,
            ln_scr, xn_scr, q8_scr, k8_scr, vt_scr, fq_scr, sk_scr, stat_scr, ot_scr, out_v,
            *rest):
    p_bufs, s_buf, sems = rest[:HB * NQ], rest[HB * NQ], rest[HB * NQ + 1]
    wt, xn, vt_all = [r.bitcast(jnp.bfloat16) for r in (wt_scr, xn_scr, vt_scr)]
    p_bufs = [r.bitcast(jnp.bfloat16) for r in p_bufs]
    step = pl.program_id(0)

    late = ((wo_hbm, wo_v), (w1_hbm, w1_v), (w3_hbm, w3_v), (w2_hbm, w2_v))

    def copy_late(n):
        return pltpu.make_async_copy(late[n][0], late[n][1], sems.at[n])

    def copy_w(n):
        cols = pl.ds(n * D, D)
        return pltpu.make_async_copy(wqkv_hbm.at[:, cols], wqkv_v.at[n], sems.at[4 + n])

    def copy_x(b):
        rows = pl.ds(pl.multiple_of(b * TQ, TQ), TQ)
        return pltpu.make_async_copy(x_hbm.at[rows, :], x_v.at[rows, :], sems.at[7 + b])

    def copy_out(blk, b):
        rows = pl.ds(pl.multiple_of(blk * TQ + b * TF, TF), TF)
        slot = (blk % 2) * (TQ // TF) + b
        return pltpu.make_async_copy(out_v.at[slot], out_hbm.at[rows, :],
                                     sems.at[7 + NQ + slot])

    def normed(sb):
        rows = pl.ds(pl.multiple_of(sb * TQ, TQ), TQ)
        ln = _layernorm_f32(x_v[rows, :].astype(jnp.float32))
        xn[0] = ln.astype(jnp.bfloat16)
        for g in range(D // 128):
            ln_scr[g] = ln[:, g * 128:(g + 1) * 128]
        xn[1] = jnp.concatenate(
            [jnp.concatenate([ln_scr[g, pl.ds(b, 128, stride=4), :]
                              for g in range(D // 128)], axis=1) for b in range(4)],
            axis=0).astype(jnp.bfloat16)

    def quantize_q(sb, h, xh):
        a = jnp.abs(xh)
        amax = jnp.max(a, axis=0, keepdims=True)
        l1 = _fold_lanes(jnp.sum(a, axis=0, keepdims=True), jnp.maximum)
        hi, x2, x1, x0, r1, r0 = _limbs(xh * (QMAX * _recip(jnp.maximum(amax, 1e-30))))
        alpha = jnp.concatenate([hi, hi, x1, x2, x1, x0, r1, r0], axis=0)
        q8_scr[sb, h] = alpha.astype(jnp.int8)
        fq_scr[sb, h] = amax * (1.0 / QMAX)
        stat_scr[0, h:h + 1, :] = jnp.maximum(stat_scr[0, h:h + 1, :], l1)

    def quantize_k(sb, h, xh):
        kmax = _splat_max(jnp.abs(xh))
        bmax = jnp.concatenate([kmax] * (TQ // 128), axis=1)
        inv = QMAX * _recip(jnp.maximum(kmax, 1e-30))
        hi, x2, x1, x0, r1, r0 = _limb_words(
            xh * jnp.concatenate([inv] * (TQ // 128), axis=1))
        words = jnp.concatenate([hi, x1, hi, x0, x1, x2, r0, r1], axis=0)
        k8_scr[h, pl.ds(pl.multiple_of(sb * 128, 128), 128), :] = words.T
        sk_scr[h * NQ + sb] = bmax * (ACC_UNIT * Q_SCALE / QMAX)
        stat_scr[1, h:h + 1, :] = jnp.maximum(stat_scr[1, h:h + 1, :], kmax)

    def project(sb):
        def proj(n):
            return lax.dot_general(wt[n * D:(n + 1) * D, :], xn[n % 2], _NT,
                                   preferred_element_type=jnp.float32)

        qt, kt = proj(0), proj(1)
        for h in range(H):
            quantize_q(sb, h, qt[h * DH:(h + 1) * DH])
        vt = proj(2)
        for h in range(H):
            quantize_k(sb, h, kt[h * DH:(h + 1) * DH])
        va = jnp.max(jnp.abs(vt).reshape(D // 8, 8, TQ), axis=0)
        stat_scr[2, 0:8, :] = jnp.maximum(stat_scr[2, 0:8, :], _fold_lanes(va, jnp.maximum))
        vt_all[sb] = vt.astype(jnp.bfloat16)

    def row_pow2(num, den):
        ok = (num > 0.0) & (den > 0.0)
        ratio = jnp.where(ok, num, 1.0) / jnp.where(ok, den, 1.0)
        e = jnp.clip(jnp.floor(0.25 * jnp.log2(ratio) + 0.5), -30.0, 30.0).astype(jnp.int32)
        return (lax.bitcast_convert_type((127 + e) << 23, jnp.float32),
                lax.bitcast_convert_type((127 - e) << 23, jnp.float32))

    def scores(c, q8, h, fs):
        k = pltpu.bitcast(k8_scr[h, c * (CK // 4):(c + 1) * (CK // 4), :], jnp.int8)
        acc = jnp.dot(k, q8, preferred_element_type=jnp.int32)
        return acc.astype(jnp.float32) * fs[(c * CK) // TQ]

    def tile_operands(h, qb):
        fq = fq_scr[qb, h]
        return q8_scr[qb, h], [fq * sk_scr[h * NQ + sb] for sb in range(NQ)]

    def values_t(h):
        rows = pl.ds(pl.multiple_of(h * DH, DH), DH)
        return jnp.concatenate([vt_all[sb, rows, :] for sb in range(NQ)], axis=1)

    def finish(h, qb, o, l8):
        l = jnp.sum(l8, axis=0, keepdims=True)
        ot_scr[qb, pl.ds(pl.multiple_of(h * DH, DH), DH), :] = o * (1.0 / l)

    def acc(total, x):
        return x if total is None else total + x

    def store_probs(c, s, l8, buf):
        p = jnp.exp2(s)
        for r in range(0, CK, 16):
            l8 = acc(l8, p[r:r + 8] + p[r + 8:r + 16])
        buf[c * CK:(c + 1) * CK, :] = p.astype(jnp.bfloat16)
        return l8

    def fast_tile(h, qb, l8, buf, prefetch):
        vt = values_t(h)
        if prefetch:
            q8, fs = tile_operands(h + HB, qb)
        o = l_next = None
        for c in range(NC):
            pb = buf[c * CK:(c + 1) * CK, :]
            if prefetch:
                s = scores(c, q8, h + HB, fs)
            for k0 in range(0, CK, PK):
                o = acc(o, jnp.dot(vt[:, c * CK + k0:c * CK + k0 + PK], pb[k0:k0 + PK],
                                   preferred_element_type=jnp.float32))
            if prefetch:
                l_next = store_probs(c, s, l_next, buf)
        finish(h, qb, o, l8)
        return l_next

    def fast_attention():
        tiles = [(j, qb) for j in range(HB) for qb in range(NQ)]
        carry = []
        for n, (j, qb) in enumerate(tiles):
            q8, fs = tile_operands(j, qb)
            l8 = None
            for c in range(NC):
                l8 = store_probs(c, scores(c, q8, j, fs), l8, p_bufs[n])
            carry.append(l8)

        def body(i, carry):
            return tuple(fast_tile(i * HB + j, qb, carry[n], p_bufs[n], True)
                         for n, (j, qb) in enumerate(tiles))

        carry = lax.fori_loop(0, H // HB - 1, body, tuple(carry))
        for n, (j, qb) in enumerate(tiles):
            fast_tile(H - HB + j, qb, carry[n], p_bufs[n], False)

    def safe_attention():
        def body(t, carry):
            h, qb = t >> 2, t & (NQ - 1)
            q8, fs = tile_operands(h, qb)
            vt = values_t(h)
            m8 = None
            for c in range(NC):
                s = scores(c, q8, h, fs)
                s_buf[c * CK:(c + 1) * CK, :] = s
                mc = jnp.max(s.reshape(CK // 8, 8, TQ), axis=0)
                m8 = mc if m8 is None else jnp.maximum(m8, mc)
            m = jnp.max(m8, axis=0, keepdims=True)
            o = l8 = None
            for c in range(NC):
                p = jnp.exp2(s_buf[c * CK:(c + 1) * CK, :] - m)
                for r in range(0, CK, 16):
                    l8 = acc(l8, p[r:r + 8] + p[r + 8:r + 16])
                o = acc(o, jnp.dot(vt[:, c * CK:(c + 1) * CK], p.astype(jnp.bfloat16),
                                   preferred_element_type=jnp.float32))
            finish(h, qb, o, l8)
            return carry

        lax.fori_loop(0, H * NQ, body, 0)

    @pl.when(step == 0)
    def _first_step():
        copy_x(0).start()
        copy_w(0).start()
        copy_w(1).start()
        copy_w(2).start()
        for b in range(1, NQ):
            copy_x(b).start()

        copy_x(0).wait()
        normed(0)
        copy_w(0).wait()
        copy_w(1).wait()
        wq_t = wqkv_v[0].astype(jnp.float32).T
        wk_t = wqkv_v[1].astype(jnp.float32).T
        cq, ck = row_pow2(jnp.sum(wk_t * wk_t, axis=1, keepdims=True),
                          jnp.sum(wq_t * wq_t, axis=1, keepdims=True))
        wt[0:D, :] = (wq_t * cq).astype(jnp.bfloat16)
        wt[D:2 * D, :] = (wk_t * ck).astype(jnp.bfloat16)
        copy_w(2).wait()
        wt[2 * D:, :] = wqkv_v[2].astype(jnp.float32).T.astype(jnp.bfloat16)

        stat_scr[...] = jnp.zeros(stat_scr.shape, jnp.float32)

        def qkv_block(sb, carry):
            nxt = jnp.minimum(sb + 1, NQ - 1)

            @pl.when(sb + 1 < NQ)
            def _():
                copy_x(nxt).wait()

            project(sb)
            normed(nxt)
            return carry

        lax.fori_loop(0, NQ, qkv_block, 0)
        for n in range(4):
            copy_late(n).start()

        bound = jnp.max(stat_scr[0] * stat_scr[1]) * Q_SCALE
        vmax = jnp.max(stat_scr[2, 0:8, :])
        no_shift_needed = (bound <= LOGIT_LIMIT) & (vmax <= V_HI) & (vmax >= V_LO)
        lax.cond(no_shift_needed, fast_attention, safe_attention)

        for n in range(4):
            copy_late(n).wait()

    @pl.when(step > 1)
    def _():
        for b in range(TQ // TF):
            copy_out(step - 2, b).wait()

    hres, hn = [], []
    for b in range(TQ // TF):
        t0 = pl.multiple_of(step * TQ + b * TF, TF)
        o = ot_scr[step, :, b * TF:(b + 1) * TF].T.astype(jnp.bfloat16)
        hb = x_v[pl.ds(t0, TF), :].astype(jnp.float32) + jnp.dot(
            o, wo_v[...], preferred_element_type=jnp.float32)
        hres.append(hb)
        hn.append(_layernorm_f32(hb).astype(jnp.bfloat16))
    for b in range(TQ // TF):
        gate = lax.dot_general(hn[b], w1_v[...], _NT, preferred_element_type=jnp.float32)
        up = lax.dot_general(hn[b], w3_v[...], _NT, preferred_element_type=jnp.float32)
        act = (gate * jax.nn.sigmoid(gate) * up).astype(jnp.bfloat16)
        ffn = jnp.dot(act, w2_v[...], preferred_element_type=jnp.float32)
        out_v[(step % 2) * (TQ // TF) + b] = (hres[b] + ffn).astype(out_v.dtype)
        copy_out(step, b).start()

    @pl.when(step == NQ - 1)
    def _():
        for b in range(TQ // TF):
            copy_out(step - 1, b).wait()
            copy_out(step, b).wait()


@jax.jit
def pallas_sequential_preLN__softmax_full_mha__glu_gated_swiglu__prompt_kernel(
    A_x: jax.Array,
    A_wqkv: jax.Array,
    A_wo: jax.Array,
    B_x: jax.Array,
    B_w1: jax.Array,
    B_w3: jax.Array,
    B_w2: jax.Array,
):
    del B_x
    bf16, f32 = jnp.bfloat16, jnp.float32
    hbm = pl.BlockSpec(memory_space=pltpu.HBM)
    out = pl.pallas_call(
        _kernel,
        grid=(NQ,),
        in_specs=[hbm] * 6,
        out_specs=hbm,
        out_shape=jax.ShapeDtypeStruct((S, D), A_x.dtype),
        scratch_shapes=[
            pltpu.VMEM((S, D), bf16),
            pltpu.VMEM((3, D, D), bf16),
            pltpu.VMEM((D, D), bf16),
            pltpu.VMEM((F, D), bf16),
            pltpu.VMEM((F, D), bf16),
            pltpu.VMEM((F, D), bf16),
            pltpu.VMEM((3 * D // 2, D), jnp.uint32),
            pltpu.VMEM((D // 128, TQ, 128), f32),
            pltpu.VMEM((2, TQ // 2, D), jnp.uint32),
            pltpu.VMEM((NQ, H, 128, TQ), jnp.int8),
            pltpu.VMEM((H, S // 4, 128), jnp.int32),
            pltpu.VMEM((NQ, D // 2, TQ), jnp.uint32),
            pltpu.VMEM((NQ, H, 1, TQ), f32),
            pltpu.VMEM((H * NQ, 1, TQ), f32),
            pltpu.VMEM((3, H, 128), f32),
            pltpu.VMEM((NQ, D, TQ), f32),
            pltpu.VMEM((2 * TQ // TF, TF, D), bf16),
            *[pltpu.VMEM((S // 2, TQ), jnp.uint32) for _ in range(HB * NQ)],
            pltpu.VMEM((S, TQ), f32),
            pltpu.SemaphoreType.DMA((7 + NQ + 2 * TQ // TF,)),
        ],
        compiler_params=pltpu.CompilerParams(
            dimension_semantics=("arbitrary",),
            vmem_limit_bytes=110 * 1024 * 1024,
        ),
    )(A_x.reshape(S, D), A_wqkv, A_wo, B_w1.T, B_w3.T, B_w2)
    return out.reshape(1, S, D)
```
